```python
import os as _os
_os.environ.setdefault("JAX_PLATFORMS", "cpu")
import jax
import jax.numpy as jnp

def _softmax(x, axis=-1):
    return jax.nn.softmax(x, axis=axis)
def _gelu(x):
    return jax.nn.gelu(x, approximate=True)
def _silu(x):
    return jax.nn.silu(x)
def _sigmoid(x):
    return jax.nn.sigmoid(x)
def _layernorm(x, axis=-1, eps=1e-5):
    m = jnp.mean(x, axis=axis, keepdims=True)
    v = jnp.var(x, axis=axis, keepdims=True)
    return (x - m) / jnp.sqrt(v + eps)
def _scatter_add(tgt, idx, src, axis=0):
    return tgt.at[idx].add(src)
def _segment_sum(src, seg, n):
    return jax.ops.segment_sum(src, seg, n)
class _Rng:
    def __init__(self, key):
        self._k = key
    def _next(self):
        self._k, sub = jax.random.split(self._k)
        return sub
    def normal(self, shape):
        return jax.random.normal(self._next(), shape, dtype=jnp.bfloat16)
    def randint(self, lo, hi, shape):
        return jax.random.randint(self._next(), shape, lo, hi, dtype=jnp.int32)
    def uniform(self, shape, lo=0.0, hi=1.0):
        return jax.random.uniform(self._next(), shape, jnp.bfloat16, lo, hi)
    def permutation(self, n):
        return jax.random.permutation(self._next(), n)


kernel_name = 'interleave_layers__sliding_local_dilated__linear_kernel_hedgehog__prompt'

def setup_inputs():
    _rng = _Rng(jax.random.key(int.from_bytes(__import__("os").urandom(4), "little")))
    _w = (lambda a: (lambda t: t.astype(jnp.bfloat16) if jnp.issubdtype(t.dtype, jnp.floating) else t)(jnp.asarray(a)))
    def _A_setup():
        B, S, D = 1, 2048, 640
        return {
            "x": _w((lambda *s: _rng.normal(s) * 0.05)(B, S, D)),
            "wqkv": _w((lambda *s: _rng.normal(s) * 0.05)(D, 3 * D)),
            "wo": _w((lambda *s: _rng.normal(s) * 0.05)(D, D)),
        }
    _A_in = _A_setup()

    def _B_setup():
        B, S, D, H = 1, 2048, 640, 32
        Dh = D // H
        return {
            "x": _w((lambda *s: _rng.normal(s) * 0.05)(B, S, D)),
            "wqkv": _w((lambda *s: _rng.normal(s) * 0.4)(D, 3 * D)),
            "w_phi": _w((lambda *s: _rng.normal(s) * 0.4)(H, Dh, Dh) * (Dh ** -0.5)),
            "wo": _w((lambda *s: _rng.normal(s) * 0.1)(D, D)),
        }
    _B_in = _B_setup()

    return {
        "A_x": _A_in["x"],
        "A_wqkv": _A_in["wqkv"],
        "A_wo": _A_in["wo"],
        "B_x": _B_in["x"],
        "B_wqkv": _B_in["wqkv"],
        "B_w_phi": _B_in["w_phi"],
        "B_wo": _B_in["wo"],
    }

def reference(A_x, A_wqkv, A_wo, B_x, B_wqkv, B_w_phi, B_wo):
    def _A_ref(x, wqkv, wo):
        B, S, D = x.shape
        H = 32; Dh = D // H
        W, dil = 8, 2
        qkv = (lambda x, *d: x.transpose(*d))((x @ wqkv).reshape(B, S, 3, H, Dh), 2, 0, 3, 1, 4)
        q, k, v = qkv[0], qkv[1], qkv[2]
        scale = Dh ** -0.5
        pos = jnp.arange(S)
        off = jnp.arange(W) * dil
        idx = pos[:, None] - off[None, :]
        mask = idx >= 0
        idx_c = jnp.where(mask, idx, 0).reshape(-1)
        kg = k[:, :, idx_c, :].reshape(B, H, S, W, Dh)
        vg = v[:, :, idx_c, :].reshape(B, H, S, W, Dh)
        logits = jnp.einsum("bhsd,bhswd->bhsw", q, kg) * scale
        logits = jnp.where(mask[None, None, :, :], logits, -1e9)
        attn = _softmax(logits, axis=-1)
        o = jnp.einsum("bhsw,bhswd->bhsd", attn, vg)
        return (lambda x, *d: x.transpose(*d))(o, 0, 2, 1, 3).reshape(B, S, D) @ wo

    def _B_ref(x, wqkv, w_phi, wo):
        B, S, D = x.shape
        H = 32; Dh = D // H
        qkv = (lambda x, *d: x.transpose(*d))((x @ wqkv).reshape(B, S, 3, H, Dh), 2, 0, 3, 1, 4)
        q, k, v = qkv[0], qkv[1], qkv[2]
        pq = jnp.einsum("bhsd,hdf->bhsf", q, w_phi)
        pk = jnp.einsum("bhsd,hdf->bhsf", k, w_phi)
        phi_q = jnp.concatenate([_softmax(pq, axis=-1), _softmax(-pq, axis=-1)], axis=-1)
        phi_k = jnp.concatenate([_softmax(pk, axis=-1), _softmax(-pk, axis=-1)], axis=-1)
        kv = jnp.einsum("bhsf,bhsd->bhfd", phi_k, v)
        z  = jnp.einsum("bhsf->bhf", phi_k)
        num = jnp.einsum("bhqf,bhfd->bhqd", phi_q, kv)
        den = jnp.einsum("bhqf,bhf->bhq", phi_q, z)[..., None] + 1e-6
        o = num / den
        return (lambda x, *d: x.transpose(*d))(o, 0, 2, 1, 3).reshape(B, S, D) @ wo

    x = A_x
    x = x + _A_ref(_layernorm(x, axis=-1), A_wqkv, A_wo)
    x = x + _B_ref(_layernorm(x, axis=-1), B_wqkv, B_w_phi, B_wo)
    x = x + _A_ref(_layernorm(x, axis=-1), A_wqkv, A_wo)
    x = x + _B_ref(_layernorm(x, axis=-1), B_wqkv, B_w_phi, B_wo)
    return x
```

```python
import jax
import jax.numpy as jnp
from jax import lax
import jax.experimental.pallas as pl
import jax.experimental.pallas.tpu as pltpu

S, D, H, DH, W, DIL = 2048, 640, 32, 20, 8, 2
NC = 16
NG, GR = 4, 160
F32, BF16 = jnp.float32, jnp.bfloat16
NT = (((1,), (1,)), ((), ()))


def _dot(a, b):
    return jnp.dot(a, b, preferred_element_type=F32)


def _kernel(x_hbm, awqkv_hbm, awo_hbm, bwqkv_hbm, wphi_ref, bwo_hbm, o_hbm,
            xio, awqkv_ref, awo_ref, bwqkv_ref, bwo_ref, sems,
            xT, hT, oT, qkv, wa, wb, woa, wob, tmp, phik, phiq, vb):

    def permuted_rows(r):
        g, d = divmod(r, DH)
        return pl.ds(g * GR + d, 8, stride=DH)

    def set_tmp(a):
        for k in range(5):
            tmp[k] = a[:, k * 128:(k + 1) * 128]

    def get_tmp(r):
        return jnp.concatenate([tmp[k, permuted_rows(r), :] for k in range(5)], axis=1)

    def put_w(dst, sec):
        for g in range(NG):
            for d in range(0, DH, 2):
                a = jnp.concatenate([get_tmp(g * DH + d), get_tmp(g * DH + d + 1)], axis=0)
                dst[pl.ds((g * 3 + sec) * GR + d * 8, 16), :] = a.astype(BF16)

    def prep_wo(src, dst):
        set_tmp(src[...].astype(F32))
        a = jnp.concatenate([get_tmp(r) for r in range(NG * DH)], axis=0)
        dst[...] = a.T.astype(BF16)

    def prep_a():
        for sec in range(3):
            set_tmp(awqkv_ref[:, sec * D:(sec + 1) * D].astype(F32).T)
            put_w(wa, sec)

    def prep_b():
        set_tmp(bwqkv_ref[:, 2 * D:3 * D].astype(F32).T)
        put_w(wb, 2)
        row = lax.broadcasted_iota(jnp.int32, (128, GR), 0)
        col = lax.broadcasted_iota(jnp.int32, (128, GR), 1)
        e = ((col // 8) == row).astype(BF16)
        row = lax.broadcasted_iota(jnp.int32, (GR, GR), 0)
        col = lax.broadcasted_iota(jnp.int32, (GR, GR), 1)
        same = (row // DH) == (col % 8)
        bds = [jnp.where(same, _dot(wphi_ref[g * GR:(g + 1) * GR, :], e), 0.0).T.astype(BF16)
               for g in range(NG)]
        for sec in range(2):
            wt = bwqkv_ref[:, sec * D:(sec + 1) * D].astype(F32).T
            for g in range(NG):
                wb[pl.ds((g * 3 + sec) * GR, GR), :] = _dot(
                    bds[g], wt[g * GR:(g + 1) * GR].astype(BF16)).astype(BF16)

    def ln(x):
        m = jnp.mean(x, axis=0, keepdims=True)
        xc = x - m
        v = jnp.mean(xc * xc, axis=0, keepdims=True)
        return (xc * lax.rsqrt(v + 1e-5)).astype(BF16)

    def load_x():
        xu = xio.bitcast(jnp.uint32)
        for c in range(0, NC, 2):
            lo, hi = [], []
            for k in range(5):
                u = xu[k, pl.ds(c // 2, 128, stride=NC // 2), :].T
                lo.append(pltpu.bitcast(u << 16, F32))
                hi.append(pltpu.bitcast(u & jnp.uint32(0xFFFF0000), F32))
            for cc, parts in ((c, lo), (c + 1, hi)):
                xc = jnp.concatenate(parts, axis=0)
                xT[:, cc * 128:(cc + 1) * 128] = xc
                hT[:, cc * 128:(cc + 1) * 128] = ln(xc)

    def out_proj(wo, last):
        CH = 256
        for j in range(S // CH):
            cs = slice(j * CH, (j + 1) * CH)
            xn = xT[:, cs] + _dot(wo[...], oT[:, cs])
            if not last:
                xT[:, cs] = xn
                hT[:, cs] = ln(xn)
            else:
                xu = xio.bitcast(jnp.uint32)
                xr = pltpu.bitcast(xn.astype(BF16).astype(F32), jnp.uint32)
                u = (xr[:, :128] >> 16) | xr[:, 128:]
                for k in range(5):
                    xu[k, pl.ds(j, 128, stride=NC // 2), :] = u[k * 128:(k + 1) * 128].T

    scale = DH ** -0.5

    def layer_a():
        for g in range(NG):
            qkv[:, 128:] = _dot(wa[pl.ds(g * 3 * GR, 3 * GR), :], hT[...])

            def blk(sec, d, j):
                rows = pl.ds(sec * GR + d * 8, 8)
                if j >= 0:
                    return qkv[rows, pl.ds(128 + j * 128, 128)]
                return pltpu.roll(qkv[rows, pl.ds(128 + (j + NC) * 128, 128)], 1, 1)

            CB = 2
            lane0 = lax.broadcasted_iota(jnp.int32, (8, 128), 1) == 0
            for c0 in [p + 2 * CB * i for p in range(2) for i in range(NC // 2 // CB)]:
                cs = [c0 + 2 * i for i in range(CB)]
                acc = {}
                for d in range(DH):
                    ks = {}
                    for c in cs:
                        q = blk(0, d, c)
                        for w in range(W):
                            j = c - DIL * w
                            if j not in ks:
                                ks[j] = blk(1, d, j)
                            p = q * ks[j]
                            acc[c, w] = p if d == 0 else acc[c, w] + p
                att = {}
                for c in cs:
                    ls = []
                    for w in range(W):
                        l = acc[c, w] * scale
                        if c - DIL * w < 0:
                            l = jnp.where(lane0, -1e9, l)
                        ls.append(l)
                    m = ls[0]
                    for l in ls[1:]:
                        m = jnp.maximum(m, l)
                    es = [jnp.exp(l - m) for l in ls]
                    s = es[0]
                    for t in es[1:]:
                        s = s + t
                    r = 1.0 / s
                    for w in range(W):
                        att[c, w] = es[w] * r
                for d in range(0, DH, 2):
                    outs = {c: [] for c in cs}
                    for dd in (d, d + 1):
                        vs = {}
                        for c in cs:
                            o = None
                            for w in range(W):
                                j = c - DIL * w
                                if j not in vs:
                                    vs[j] = blk(2, dd, j)
                                p = att[c, w] * vs[j]
                                o = p if o is None else o + p
                            outs[c].append(o)
                    for c in cs:
                        oT[pl.ds(g * GR + d * 8, 16), pl.ds(c * 128, 128)] = (
                            jnp.concatenate(outs[c], axis=0).astype(BF16))

    def layer_b():
        r_ = lax.broadcasted_iota(jnp.int32, (GR + 16, 2 * GR), 0)
        c_ = lax.broadcasted_iota(jnp.int32, (GR + 16, 2 * GR), 1)
        diag = (r_ % 8) == (c_ % 8)
        for g in range(NG):
            qkv[:, 128:] = _dot(wb[pl.ds(g * 3 * GR, 3 * GR), :], hT[...])
            vb[:GR, :] = qkv[2 * GR:, 128:].astype(BF16)
            for sec, dst in ((1, phik), (0, phiq)):
                for c in range(NC):
                    cs = pl.ds(128 + c * 128, 128)
                    p = [qkv[pl.ds(sec * GR + d * 8, 8), cs] for d in range(DH)]
                    mx, mn = p[0], p[0]
                    for t in p[1:]:
                        mx = jnp.maximum(mx, t)
                        mn = jnp.minimum(mn, t)
                    for half_, es in enumerate(([jnp.exp(t - mx) for t in p],
                                                [jnp.exp(mn - t) for t in p])):
                        s = es[0]
                        for t in es[1:]:
                            s = s + t
                        r = 1.0 / s
                        dst[pl.ds(half_ * GR, GR), pl.ds(c * 128, 128)] = (
                            jnp.concatenate([t * r for t in es], axis=0).astype(BF16))
            kv = lax.dot_general(vb[...], phik[...], NT, preferred_element_type=F32)
            kv = jnp.where(diag, kv, 0.0).astype(BF16)
            CH = 512
            for j in range(S // CH):
                cs = slice(j * CH, (j + 1) * CH)
                nd = _dot(kv, phiq[:, cs])
                r = 1.0 / (nd[GR:GR + 8] + 1e-6)
                o = nd[:GR].reshape(DH, 8, CH) * r[None]
                oT[pl.ds(g * GR, GR), cs] = o.reshape(GR, CH).astype(BF16)

    def xcopy(k, out, sem):
        hb = (o_hbm if out else x_hbm).at[:, pl.ds(k * 128, 128)]
        return (pltpu.make_async_copy(xio.at[k], hb, sem) if out
                else pltpu.make_async_copy(hb, xio.at[k], sem))

    xin = [xcopy(k, False, sems.at[0]) for k in range(5)]
    wcp = [pltpu.make_async_copy(s_, d_, sems.at[1 + i]) for i, (s_, d_) in enumerate(
        ((awqkv_hbm, awqkv_ref), (awo_hbm, awo_ref), (bwqkv_hbm, bwqkv_ref), (bwo_hbm, bwo_ref)))]
    for c_ in xin:
        c_.start()
    wcp[0].start()
    vb[GR:, :] = jnp.ones((16, S), BF16)
    for c_ in xin:
        c_.wait()
    with jax.named_scope("ldx"):
        load_x()
    wcp[0].wait()
    for c_ in wcp[1:]:
        c_.start()
    with jax.named_scope("wa"):
        prep_a()
    for i in range(2):
        with jax.named_scope("la"):
            layer_a()
        if i == 0:
            with jax.named_scope("wb"):
                for c_ in wcp[1:]:
                    c_.wait()
                prep_wo(awo_ref, woa)
                prep_wo(bwo_ref, wob)
                prep_b()
        with jax.named_scope("oa"):
            out_proj(woa, False)
        with jax.named_scope("lb"):
            layer_b()
        with jax.named_scope("ob"):
            out_proj(wob, i == 1)

    xout = [xcopy(k, True, sems.at[5]) for k in range(5)]
    for c_ in xout:
        c_.start()
    for c_ in xout:
        c_.wait()


@jax.jit
def pallas_interleave_layers__sliding_local_dilated__linear_kernel_hedgehog__prompt_kernel(
    A_x, A_wqkv, A_wo, B_x, B_wqkv, B_w_phi, B_wo,
):
    wphi = jnp.pad(B_w_phi.reshape(D, DH), ((0, 0), (0, 128 - DH)))
    out = pl.pallas_call(
        _kernel,
        out_shape=jax.ShapeDtypeStruct((S, D), BF16),
        in_specs=[pl.BlockSpec(memory_space=pl.ANY)] * 4
        + [pl.BlockSpec(memory_space=pltpu.VMEM), pl.BlockSpec(memory_space=pl.ANY)],
        out_specs=pl.BlockSpec(memory_space=pl.ANY),
        scratch_shapes=[
            pltpu.VMEM((5, S, 128), BF16),
            pltpu.VMEM((D, 3 * D), BF16),
            pltpu.VMEM((D, D), BF16),
            pltpu.VMEM((D, 3 * D), BF16),
            pltpu.VMEM((D, D), BF16),
            pltpu.SemaphoreType.DMA((6,)),
            pltpu.VMEM((D, S), F32),
            pltpu.VMEM((D, S), BF16),
            pltpu.VMEM((D, S), BF16),
            pltpu.VMEM((3 * GR, S + 128), F32),
            pltpu.VMEM((3 * D, D), BF16),
            pltpu.VMEM((3 * D, D), BF16),
            pltpu.VMEM((D, D), BF16),
            pltpu.VMEM((D, D), BF16),
            pltpu.VMEM((5, D, 128), F32),
            pltpu.VMEM((2 * GR, S), BF16),
            pltpu.VMEM((2 * GR, S), BF16),
            pltpu.VMEM((GR + 16, S), BF16),
        ],
        compiler_params=pltpu.CompilerParams(vmem_limit_bytes=100 * 1024 * 1024),
    )(A_x.reshape(S, D), A_wqkv, A_wo, B_wqkv, wphi, B_wo)
    return out.reshape(1, S, D)
```
